```python
import jax
import jax.numpy as jnp

def _softmax(x, axis=-1):
    return jax.nn.softmax(x, axis=axis)
def _gelu(x):
    return jax.nn.gelu(x, approximate=True)
def _silu(x):
    return jax.nn.silu(x)
def _sigmoid(x):
    return jax.nn.sigmoid(x)
def _layernorm(x, axis=-1, eps=1e-5):
    m = jnp.mean(x, axis=axis, keepdims=True)
    v = jnp.var(x, axis=axis, keepdims=True)
    return (x - m) / jnp.sqrt(v + eps)
def _scatter_add(tgt, idx, src, axis=0):
    return tgt.at[idx].add(src)
def _segment_sum(src, seg, n):
    return jax.ops.segment_sum(src, seg, n)
class _Rng:
    def __init__(self, key):
        self._k = key
    def _next(self):
        self._k, sub = jax.random.split(self._k)
        return sub
    def normal(self, shape):
        return jax.random.normal(self._next(), shape, dtype=jnp.bfloat16)
    def randint(self, lo, hi, shape):
        return jax.random.randint(self._next(), shape, lo, hi, dtype=jnp.int32)
    def uniform(self, shape, lo=0.0, hi=1.0):
        return jax.random.uniform(self._next(), shape, jnp.bfloat16, lo, hi)
    def permutation(self, n):
        return jax.random.permutation(self._next(), n)


kernel_name = 'standalone__layerscale__sampling'

def _fwd_setup_inputs():
    _rng = _Rng(jax.random.key(int.from_bytes(__import__("os").urandom(4), "little")))
    _w = (lambda a: (lambda t: t.astype(jnp.bfloat16) if jnp.issubdtype(t.dtype, jnp.floating) else t)(jnp.asarray(a)))
    B, S, D = 1024, 8, 512
    return {
        "x": _w((lambda *s: _rng.normal(s) * 0.05)(B, S, D)),
        "y": _w((lambda *s: _rng.normal(s) * 0.05)(B, S, D)),
        "gamma": _w(1e-4 * (lambda *s: _rng.normal(s) * 0.05)(D)),
    }

def _fwd_reference(x, y, gamma):
    return x + gamma * y


def setup_inputs():
    _inp = _fwd_setup_inputs()
    _gk = jax.random.fold_in(jax.random.key(int.from_bytes(__import__("os").urandom(4), "little")), 2**31 - 1)
    _shapes = [[1024, 8, 512]]
    _dtypes = ['bfloat16']
    _gks = jax.random.split(_gk, len(_shapes))
    _gs = [jax.random.normal(k, s, dtype=jnp.dtype(d)) * 0.05 for k, s, d in zip(_gks, _shapes, _dtypes)]
    _inp["grad_out"] = _gs[0]
    return _inp

def reference(x, y, gamma, grad_out):
    _const = dict()
    def _f(*_d):
        return _fwd_reference(**{'x': _d[0], 'y': _d[1], 'gamma': _d[2], **_const})
    _out, _vjp = jax.vjp(_f, x, y, gamma)
    _grads = _vjp(grad_out)
    _out0 = jnp.asarray(_out)
    return (_out0, *[jnp.asarray(_g) for _g in _grads])
```

```python
import jax
import jax.numpy as jnp
from jax import lax
import jax.experimental.pallas as pl
import jax.experimental.pallas.tpu as pltpu

NS = 8
RD_M = 2
RD_R = 2
WR_R = 2
TAIL = 6
LANES = 128


def _kernel(x_hbm, y_hbm, gm_hbm, g_hbm, o_hbm, gx_hbm, gy_hbm, gg_hbm,
            xb, yb, gb, ob, gyb, gmb, ggb, sems):
    f32 = jnp.float32
    _, nb, s, d = xb.shape
    nrd = nb // RD_R
    nwr = nb // WR_R
    sem_x, sem_y, sem_g, sem_w, sem_m, sem_t = (sems.at[i] for i in range(6))

    def wait_bytes_of(ref, sem):
        pltpu.make_async_copy(ref, ref, sem).wait()

    gm_cp = pltpu.make_async_copy(gm_hbm, gmb, sem_m)
    gm_cp.start()

    def read(src, dst, sem, lo, hi):
        def body(i, carry):
            for p in range(NS // RD_M):
                sl = (pl.ds(p * RD_M, RD_M), pl.ds(i * RD_R, RD_R))
                pltpu.make_async_copy(src.at[sl], dst.at[sl], sem).start(priority=p % 2)
            return carry
        lax.fori_loop(lo, hi, body, 0)

    read(g_hbm, gb, sem_g, 0, nrd)
    read(y_hbm, yb, sem_y, 0, nrd)
    read(x_hbm, xb, sem_x, 0, nrd - TAIL)
    read(x_hbm, xb, sem_t, nrd - TAIL, nrd)
    gm_cp.wait()
    wait_bytes_of(gb, sem_g)
    wait_bytes_of(yb, sem_y)
    head = (nrd - TAIL) * RD_R
    wait_bytes_of(xb.at[:, pl.ds(0, head)], sem_x)

    def write(src, dst, c):
        sl = (slice(None), pl.ds(c * WR_R, WR_R))
        pltpu.make_async_copy(src.at[sl], dst.at[sl], sem_w).start()

    def gx_body(c, carry):
        write(gb, gx_hbm, c)
        return carry
    lax.fori_loop(0, nwr, gx_body, 0)
    wait_bytes_of(xb.at[:, pl.ds(head, nb - head)], sem_t)

    gm_rows = gmb[...].astype(f32)
    gm = jnp.concatenate(
        [jnp.broadcast_to(gm_rows[j:j + 1], (s, LANES)) for j in range(d // LANES)],
        axis=1)

    def gy_body(c, acc):
        for p in range(NS):
            for q in range(WR_R):
                g = gb[p, c * WR_R + q].astype(f32)
                y = yb[p, c * WR_R + q].astype(f32)
                gyb[p, c * WR_R + q] = (g * gm).astype(gyb.dtype)
                acc = acc + g * y
        write(gyb, gy_hbm, c)
        return acc
    acc = lax.fori_loop(0, nwr, gy_body, jnp.zeros((s, d), f32))

    tot = jnp.sum(acc, axis=0, keepdims=True)
    ggb[...] = jnp.concatenate(
        [tot[:, j * LANES:(j + 1) * LANES] for j in range(d // LANES)],
        axis=0).astype(ggb.dtype)
    gg_cp = pltpu.make_async_copy(ggb, gg_hbm, sem_m)
    gg_cp.start()

    def out_body(c, carry):
        for p in range(NS):
            for q in range(WR_R):
                x = xb[p, c * WR_R + q].astype(f32)
                y = yb[p, c * WR_R + q].astype(f32)
                ob[p, c * WR_R + q] = (x + gm * y).astype(ob.dtype)
        write(ob, o_hbm, c)
        return carry
    lax.fori_loop(0, nwr, out_body, 0)

    gg_cp.wait()
    wait_bytes_of(gb, sem_w)
    wait_bytes_of(gyb, sem_w)
    wait_bytes_of(ob, sem_w)


@jax.jit
def pallas_standalone__layerscale__sampling_kernel(
    x: jax.Array,
    y: jax.Array,
    gamma: jax.Array,
    grad_out: jax.Array,
):
    b, s, d = x.shape
    shp = (NS, b // NS, s, d)
    gshp = (d // LANES, LANES)
    hbm = pl.BlockSpec(memory_space=pl.ANY)
    big = jax.ShapeDtypeStruct(shp, x.dtype)
    out, gx, gy, gg = pl.pallas_call(
        _kernel,
        in_specs=[hbm] * 4,
        out_specs=[hbm] * 4,
        out_shape=[big, big, big, jax.ShapeDtypeStruct(gshp, gamma.dtype)],
        scratch_shapes=(
            [pltpu.VMEM(shp, x.dtype)] * 5
            + [pltpu.VMEM(gshp, gamma.dtype)] * 2
            + [pltpu.SemaphoreType.DMA((6,))]
        ),
        compiler_params=pltpu.CompilerParams(vmem_limit_bytes=64 * 1024 * 1024),
    )(x.reshape(shp), y.reshape(shp), gamma.reshape(gshp), grad_out.reshape(shp))
    return out.reshape(x.shape), gx.reshape(x.shape), gy.reshape(x.shape), gg.reshape(d)
```

```python
import jax
import jax.numpy as jnp
from jax import lax
import jax.experimental.pallas as pl
import jax.experimental.pallas.tpu as pltpu

LANES = 128
STREAMS = 8
LEAD = 13
TAIL = 3
WCOLS = 2


def _body(x_hbm, y_hbm, gm_hbm, g_hbm, o_hbm, gx_hbm, gy_hbm, gg_hbm,
          xb, yb, gb, ob, gyb, gmb, ggb, sems):
    f32 = jnp.float32
    _, _, ncol, s, d = xb.shape
    (sem_g, sem_y, sem_x, sem_xtail, sem_gm,
     sem_gx, sem_gy, sem_o, sem_gg) = (sems.at[i] for i in range(9))

    def wait_filled(buf, sem):
        pltpu.make_async_copy(buf, buf, sem).wait()

    inputs = ((g_hbm, gb, sem_g), (y_hbm, yb, sem_y), (x_hbm, xb, sem_x))

    def read(src, dst, sem, half, col, lane0, nlane, priority):
        idx = (slice(None), half, pl.ds(col, 1), slice(None), pl.ds(lane0, nlane))
        pltpu.make_async_copy(src.at[idx], dst.at[idx], sem).start(priority=priority)

    def read_big(a, col, j, priority):
        read(*inputs[a], 1 - priority, col, j * (d // 2), d // 2, priority)

    def read_cols(n, a1, col1, a0=None, col0=None):
        def step(k, carry):
            for j in range(2):
                read_big(a1, col1 + k, j, 1)
                if a0 is not None:
                    read_big(a0, col0 + k, j, 0)
            return carry
        lax.fori_loop(0, n, step, 0)

    gm_copy = pltpu.make_async_copy(gm_hbm, gmb, sem_gm)
    head = ncol - TAIL
    read_cols(LEAD, 0, 0)
    gm_copy.start()
    read_cols(ncol - LEAD, 0, LEAD, 0, 0)
    read_cols(LEAD, 1, 0, 0, ncol - LEAD)
    read_cols(ncol - LEAD, 1, LEAD, 1, 0)
    read_cols(LEAD, 2, 0, 1, ncol - LEAD)
    read_cols(head - LEAD, 2, LEAD, 2, 0)
    small = [(half, col, lane0)
             for col in range(head, ncol)
             for lane0 in range(0, d, LANES)
             for half in range(2)]
    rest = [(col, j) for col in range(head - LEAD, head) for j in range(2)]
    for k in range(max(len(small), len(rest))):
        if k < len(small):
            read(x_hbm, xb, sem_xtail, *small[k], LANES, 1)
        if k < len(rest):
            read_big(2, *rest[k], 0)

    gm_copy.wait()
    wait_filled(gb, sem_g)
    wait_filled(yb, sem_y)
    wait_filled(xb.at[:, :, pl.ds(0, head)], sem_x)

    def for_each_chunk(fn, init):
        def over_half(half, carry):
            return lax.fori_loop(
                0, ncol // WCOLS, lambda c, cr: fn(half, c * WCOLS, cr), carry)
        return lax.fori_loop(0, 2, over_half, init)

    def write(src, dst, sem, half, col):
        idx = (slice(None), half, pl.ds(col, WCOLS))
        pltpu.make_async_copy(src.at[idx], dst.at[idx], sem).start()

    def gx_chunk(half, col, carry):
        write(gb, gx_hbm, sem_gx, half, col)
        return carry
    for_each_chunk(gx_chunk, 0)

    wait_filled(xb.at[:, :, pl.ds(head, TAIL)], sem_xtail)

    gm_rows = gmb[...].astype(f32)
    gm = jnp.concatenate(
        [jnp.broadcast_to(gm_rows[j:j + 1], (s, LANES)) for j in range(d // LANES)],
        axis=1)

    def gy_chunk(half, col, acc):
        for p in range(STREAMS):
            for q in range(WCOLS):
                g = gb[p, half, col + q].astype(f32)
                y = yb[p, half, col + q].astype(f32)
                gyb[p, half, col + q] = (g * gm).astype(gyb.dtype)
                acc = acc + g * y
        write(gyb, gy_hbm, sem_gy, half, col)
        return acc
    acc = for_each_chunk(gy_chunk, jnp.zeros((s, d), f32))

    total = jnp.sum(acc, axis=0, keepdims=True)
    ggb[...] = jnp.concatenate(
        [total[:, j * LANES:(j + 1) * LANES] for j in range(d // LANES)],
        axis=0).astype(ggb.dtype)
    gg_copy = pltpu.make_async_copy(ggb, gg_hbm, sem_gg)
    gg_copy.start()

    def out_chunk(half, col, carry):
        for p in range(STREAMS):
            for q in range(WCOLS):
                x = xb[p, half, col + q].astype(f32)
                y = yb[p, half, col + q].astype(f32)
                ob[p, half, col + q] = (x + gm * y).astype(ob.dtype)
        write(ob, o_hbm, sem_o, half, col)
        return carry
    for_each_chunk(out_chunk, 0)

    wait_filled(gx_hbm, sem_gx)
    wait_filled(gy_hbm, sem_gy)
    gg_copy.wait()
    wait_filled(o_hbm, sem_o)


def _kernel(*refs):
    pl.run_scoped(lambda sems: _body(*refs, sems), pltpu.SemaphoreType.DMA((9,)))


@jax.jit
def pallas_standalone__layerscale__sampling_kernel(
    x: jax.Array,
    y: jax.Array,
    gamma: jax.Array,
    grad_out: jax.Array,
):
    b, s, d = x.shape
    shape = (STREAMS, 2, b // (2 * STREAMS), s, d)
    gshape = (d // LANES, LANES)
    hbm = pl.BlockSpec(memory_space=pl.ANY)
    big = jax.ShapeDtypeStruct(shape, x.dtype)
    out, grad_x, grad_y, grad_gamma = pl.pallas_call(
        _kernel,
        in_specs=[hbm] * 4,
        out_specs=[hbm] * 4,
        out_shape=[big, big, big, jax.ShapeDtypeStruct(gshape, gamma.dtype)],
        scratch_shapes=(
            [pltpu.VMEM(shape, x.dtype)] * 5 + [pltpu.VMEM(gshape, gamma.dtype)] * 2
        ),
        compiler_params=pltpu.CompilerParams(vmem_limit_bytes=64 * 1024 * 1024),
    )(x.reshape(shape), y.reshape(shape), gamma.reshape(gshape), grad_out.reshape(shape))
    return (out.reshape(x.shape), grad_x.reshape(x.shape), grad_y.reshape(x.shape),
            grad_gamma.reshape(d))
```

```python
import jax
import jax.numpy as jnp
from jax import lax
import jax.experimental.pallas as pl
import jax.experimental.pallas.tpu as pltpu

LANES = 128
STREAMS = 8
SPLIT = 2
LEAD = 26
TAIL = 4
WCOLS = 2

READ_GROUPS = (
    (("g", 0, STREAMS - SPLIT),),
    (("g", STREAMS - SPLIT, SPLIT), ("y", 0, STREAMS), ("x_lo", 0, SPLIT)),
    (("x_head", SPLIT, STREAMS - SPLIT),),
)
WRITE_GROUPS = (
    (("gx", SPLIT, STREAMS - SPLIT),),
    (("gy", 0, SPLIT), ("gx", 0, SPLIT), ("out", 0, SPLIT)),
    (("gy", SPLIT, STREAMS - SPLIT),),
    (("out", SPLIT, STREAMS - SPLIT),),
)
SEMS = ("g", "y", "x_lo", "x_head", "x_tail", "gm", "gx", "gy", "out", "gg")


def _read_order(ncol, d):
    def descriptors(priority, group, halves, cols, nlane):
        return [(priority, *part, half, lane0, nlane, col)
                for col in cols for lane0 in range(0, d, nlane)
                for half in halves for part in group]

    lo, hi = [], []
    for group in READ_GROUPS:
        cols = range(ncol - TAIL if group is READ_GROUPS[-1] else ncol)
        lo += descriptors(1, group, (0,), cols, d // 2)
        hi += descriptors(0, group, (1,), cols, d // 2)
    lo += descriptors(1, (("x_tail", SPLIT, STREAMS - SPLIT),), (0, 1),
                      range(ncol - TAIL, ncol), LANES)
    order = lo[:LEAD]
    for k in range(max(len(lo) - LEAD, len(hi))):
        order += lo[LEAD + k:LEAD + k + 1] + hi[k:k + 1]
    return order


def _roll_loops(order):
    def trips(i, period):
        body = order[i:i + period]
        nxt = order[i + period:i + 2 * period]
        if len(nxt) < period:
            return 1, [0] * period
        steps = [b[-1] - a[-1] for a, b in zip(body, nxt)]
        n = 1
        while order[i + n * period:i + (n + 1) * period] == [
                (*a[:-1], a[-1] + n * st) for a, st in zip(body, steps)]:
            n += 1
        return n, steps

    loops, i = [], 0
    while i < len(order):
        period, (n, steps) = 1, (1, [0])
        for p in (2, 4, 12, 16):
            m, st = trips(i, p)
            if m >= 3 and m * p > n * period:
                period, n, steps = p, m, st
        loops.append((order[i:i + period], steps, n))
        i += n * period
    return loops


def _body(x_hbm, y_hbm, gm_hbm, g_hbm, o_hbm, gx_hbm, gy_hbm, gg_hbm,
          xb, yb, gb, ob, gyb, gmb, ggb, sems):
    f32 = jnp.float32
    _, _, ncol, s, d = xb.shape
    sem = {name: sems.at[i] for i, name in enumerate(SEMS)}
    copies = {
        "g": (g_hbm, gb), "y": (y_hbm, yb),
        "x_lo": (x_hbm, xb), "x_head": (x_hbm, xb), "x_tail": (x_hbm, xb),
        "gx": (gb, gx_hbm), "gy": (gyb, gy_hbm), "out": (ob, o_hbm),
    }

    def start(name, idx, priority=0):
        src, dst = copies[name]
        pltpu.make_async_copy(src.at[idx], dst.at[idx], sem[name]).start(priority=priority)

    def wait_filled(name, buf):
        pltpu.make_async_copy(buf, buf, sem[name]).wait()

    def read(desc, shift):
        priority, name, s0, ns, half, lane0, nlane, col = desc
        start(name, (pl.ds(s0, ns), half, pl.ds(col + shift, 1), slice(None),
                     pl.ds(lane0, nlane)), priority)

    gm_copy = pltpu.make_async_copy(gm_hbm, gmb, sem["gm"])
    for i, (descs, steps, n) in enumerate(_roll_loops(_read_order(ncol, d))):
        if n == 1:
            read(descs[0], 0)
        else:
            def issue(k, carry, descs=descs, steps=steps):
                for desc, st in zip(descs, steps):
                    read(desc, k * st)
                return carry
            lax.fori_loop(0, n, issue, 0)
        if i == 0:
            gm_copy.start()

    gm_copy.wait()
    gm_rows = gmb[...].astype(f32)
    gm = jnp.concatenate(
        [jnp.broadcast_to(gm_rows[j:j + 1], (s, LANES)) for j in range(d // LANES)],
        axis=1)

    upper = pl.ds(SPLIT, STREAMS - SPLIT)
    wait_filled("g", gb)
    wait_filled("y", yb)
    wait_filled("x_lo", xb.at[pl.ds(0, SPLIT)])
    wait_filled("x_head", xb.at[upper, :, pl.ds(0, ncol - TAIL)])

    def write_group(group, acc):
        def chunk(half, col, acc):
            for name, s0, ns in group:
                for p in range(s0, s0 + ns):
                    for c in range(WCOLS):
                        at = (p, half, col + c)
                        if name == "gy":
                            g = gb[at].astype(f32)
                            gyb[at] = (g * gm).astype(gyb.dtype)
                            acc = acc + g * yb[at].astype(f32)
                        elif name == "out":
                            ob[at] = (xb[at].astype(f32)
                                      + gm * yb[at].astype(f32)).astype(ob.dtype)
                start(name, (pl.ds(s0, ns), half, pl.ds(col, WCOLS)))
            return acc

        def over_half(half, acc):
            return lax.fori_loop(
                0, ncol // WCOLS, lambda k, a: chunk(half, k * WCOLS, a), acc)
        return lax.fori_loop(0, 2, over_half, acc)

    write_group(WRITE_GROUPS[0], 0)
    wait_filled("x_tail", xb.at[upper, :, pl.ds(ncol - TAIL, TAIL)])
    acc = write_group(WRITE_GROUPS[1], jnp.zeros((s, d), f32))
    acc = write_group(WRITE_GROUPS[2], acc)

    total = jnp.sum(acc, axis=0, keepdims=True)
    ggb[...] = jnp.concatenate(
        [total[:, j * LANES:(j + 1) * LANES] for j in range(d // LANES)],
        axis=0).astype(ggb.dtype)
    gg_copy = pltpu.make_async_copy(ggb, gg_hbm, sem["gg"])
    gg_copy.start()

    write_group(WRITE_GROUPS[3], 0)

    wait_filled("gx", gx_hbm)
    wait_filled("gy", gy_hbm)
    gg_copy.wait()
    wait_filled("out", o_hbm)


def _kernel(*refs):
    pl.run_scoped(lambda sems: _body(*refs, sems),
                  pltpu.SemaphoreType.DMA((len(SEMS),)))


@jax.jit
def pallas_standalone__layerscale__sampling_kernel(
    x: jax.Array,
    y: jax.Array,
    gamma: jax.Array,
    grad_out: jax.Array,
):
    b, s, d = x.shape
    shape = (STREAMS, 2, b // (2 * STREAMS), s, d)
    gshape = (d // LANES, LANES)
    hbm = pl.BlockSpec(memory_space=pl.ANY)
    big = jax.ShapeDtypeStruct(shape, x.dtype)
    out, grad_x, grad_y, grad_gamma = pl.pallas_call(
        _kernel,
        in_specs=[hbm] * 4,
        out_specs=[hbm] * 4,
        out_shape=[big, big, big, jax.ShapeDtypeStruct(gshape, gamma.dtype)],
        scratch_shapes=(
            [pltpu.VMEM(shape, x.dtype)] * 5 + [pltpu.VMEM(gshape, gamma.dtype)] * 2
        ),
        compiler_params=pltpu.CompilerParams(vmem_limit_bytes=64 * 1024 * 1024),
    )(x.reshape(shape), y.reshape(shape), gamma.reshape(gshape), grad_out.reshape(shape))
    return (out.reshape(x.shape), grad_x.reshape(x.shape), grad_y.reshape(x.shape),
            grad_gamma.reshape(d))
```

```python
import jax
import jax.numpy as jnp
from jax import lax
import jax.experimental.pallas as pl
import jax.experimental.pallas.tpu as pltpu

LANES = 128
STREAMS = 8
SPLIT = 2
LEAD = 26
TAIL = 4
WCOLS = 2

READ_GROUPS = (
    (("g", 0, STREAMS - SPLIT),),
    (("g", STREAMS - SPLIT, SPLIT), ("y", 0, STREAMS), ("x_lo", 0, SPLIT)),
    (("x_head", SPLIT, STREAMS - SPLIT),),
)
WRITE_GROUPS = (
    (("gx", SPLIT, STREAMS - SPLIT),),
    (("gy", STREAMS - SPLIT, SPLIT), ("gx", 0, SPLIT), ("out", 0, SPLIT)),
    (("gy", 0, STREAMS - SPLIT),),
    (("out", SPLIT, STREAMS - SPLIT),),
)
SEMS = ("g", "y", "x_lo", "x_head", "x_edge0", "x_edge1", "x_tail", "gm",
        "gx", "gy", "out", "gg")


def _read_order(ncol, d):
    def descriptors(priority, group, halves, cols, nlane):
        return [(priority, *part, half, lane0, nlane, col)
                for col in cols for lane0 in range(0, d, nlane)
                for half in halves for part in group]

    lo, hi = [], []
    for group in READ_GROUPS:
        cols = range(ncol - TAIL if group is READ_GROUPS[-1] else ncol)
        lo += descriptors(1, group, (0,), cols, d // 2)
        hi += descriptors(0, group, (1,), cols, d // 2)
    for queue in (lo, hi):
        for k, name in ((-2, "x_edge0"), (-1, "x_edge1")):
            queue[k] = (queue[k][0], name, *queue[k][2:])
    lo += descriptors(1, (("x_tail", SPLIT, STREAMS - SPLIT),), (0, 1),
                      range(ncol - TAIL, ncol), LANES)
    order = lo[:LEAD]
    for k in range(max(len(lo) - LEAD, len(hi))):
        order += lo[LEAD + k:LEAD + k + 1] + hi[k:k + 1]
    return order


def _roll_loops(order):
    def trips(i, period):
        body = order[i:i + period]
        nxt = order[i + period:i + 2 * period]
        if len(nxt) < period:
            return 1, [0] * period
        steps = [b[-1] - a[-1] for a, b in zip(body, nxt)]
        n = 1
        while order[i + n * period:i + (n + 1) * period] == [
                (*a[:-1], a[-1] + n * st) for a, st in zip(body, steps)]:
            n += 1
        return n, steps

    loops, i = [], 0
    while i < len(order):
        period, (n, steps) = 1, (1, [0])
        for p in (2, 4, 12, 16):
            m, st = trips(i, p)
            if m >= 3 and m * p > n * period:
                period, n, steps = p, m, st
        loops.append((order[i:i + period], steps, n))
        i += n * period
    return loops


def _body(x_hbm, y_hbm, gm_hbm, g_hbm, o_hbm, gx_hbm, gy_hbm, gg_hbm,
          xb, yb, gb, ob, gyb, gmb, ggb, sems):
    f32 = jnp.float32
    _, _, ncol, s, d = xb.shape
    sem = {name: sems.at[i] for i, name in enumerate(SEMS)}
    copies = {
        "g": (g_hbm, gb), "y": (y_hbm, yb),
        "gx": (gb, gx_hbm), "gy": (gyb, gy_hbm), "out": (ob, o_hbm),
        **{name: (x_hbm, xb) for name in SEMS if name.startswith("x_")},
    }

    def start(name, idx, priority=0):
        src, dst = copies[name]
        pltpu.make_async_copy(src.at[idx], dst.at[idx], sem[name]).start(priority=priority)

    def wait_filled(name, buf):
        pltpu.make_async_copy(buf, buf, sem[name]).wait()

    def read(desc, shift):
        priority, name, s0, ns, half, lane0, nlane, col = desc
        start(name, (pl.ds(s0, ns), half, pl.ds(col + shift, 1), slice(None),
                     pl.ds(lane0, nlane)), priority)

    gm_copy = pltpu.make_async_copy(gm_hbm, gmb, sem["gm"])
    for i, (descs, steps, n) in enumerate(_roll_loops(_read_order(ncol, d))):
        if n == 1:
            read(descs[0], 0)
        else:
            def issue(k, carry, descs=descs, steps=steps):
                for desc, st in zip(descs, steps):
                    read(desc, k * st)
                return carry
            lax.fori_loop(0, n, issue, 0)
        if i == 0:
            gm_copy.start()

    gm_copy.wait()
    gm_rows = gmb[...].astype(f32)
    gm = jnp.concatenate(
        [jnp.broadcast_to(gm_rows[j:j + 1], (s, LANES)) for j in range(d // LANES)],
        axis=1)

    upper = pl.ds(SPLIT, STREAMS - SPLIT)
    edge = ncol - TAIL - 1
    wait_filled("g", gb)
    wait_filled("y", yb)
    wait_filled("x_lo", xb.at[pl.ds(0, SPLIT)])
    wait_filled("x_head", xb.at[upper, :, pl.ds(0, edge)])
    wait_filled("x_edge0", xb.at[upper, :, pl.ds(edge, 1), :, pl.ds(0, d // 2)])

    def write_group(group, acc):
        def chunk(half, col, acc):
            for name, s0, ns in group:
                at = (pl.ds(s0, ns), half, pl.ds(col, WCOLS))
                if name == "gy":
                    g = gb[at].astype(f32)
                    gyb[at] = (g * gm).astype(gyb.dtype)
                    acc = acc + jnp.sum(g * yb[at].astype(f32), axis=(0, 1))
                elif name == "out":
                    ob[at] = (xb[at].astype(f32)
                              + gm * yb[at].astype(f32)).astype(ob.dtype)
                start(name, at)
            return acc

        def over_half(half, acc):
            return lax.fori_loop(
                0, ncol // WCOLS, lambda k, a: chunk(half, k * WCOLS, a), acc)
        return lax.fori_loop(0, 2, over_half, acc)

    write_group(WRITE_GROUPS[0], 0)
    wait_filled("x_edge1", xb.at[upper, :, pl.ds(edge, 1), :, pl.ds(d // 2, d // 2)])
    wait_filled("x_tail", xb.at[upper, :, pl.ds(edge + 1, TAIL)])
    acc = write_group(WRITE_GROUPS[1], jnp.zeros((s, d), f32))
    acc = write_group(WRITE_GROUPS[2], acc)

    total = jnp.sum(acc, axis=0, keepdims=True)
    ggb[...] = jnp.concatenate(
        [total[:, j * LANES:(j + 1) * LANES] for j in range(d // LANES)],
        axis=0).astype(ggb.dtype)
    gg_copy = pltpu.make_async_copy(ggb, gg_hbm, sem["gg"])
    gg_copy.start()

    write_group(WRITE_GROUPS[3], 0)

    wait_filled("gx", gx_hbm)
    wait_filled("gy", gy_hbm)
    gg_copy.wait()
    wait_filled("out", o_hbm)


def _kernel(*refs):
    pl.run_scoped(lambda sems: _body(*refs, sems),
                  pltpu.SemaphoreType.DMA((len(SEMS),)))


@jax.jit
def pallas_standalone__layerscale__sampling_kernel(
    x: jax.Array,
    y: jax.Array,
    gamma: jax.Array,
    grad_out: jax.Array,
):
    b, s, d = x.shape
    shape = (STREAMS, 2, b // (2 * STREAMS), s, d)
    gshape = (d // LANES, LANES)
    hbm = pl.BlockSpec(memory_space=pl.ANY)
    big = jax.ShapeDtypeStruct(shape, x.dtype)
    out, grad_x, grad_y, grad_gamma = pl.pallas_call(
        _kernel,
        in_specs=[hbm] * 4,
        out_specs=[hbm] * 4,
        out_shape=[big, big, big, jax.ShapeDtypeStruct(gshape, gamma.dtype)],
        scratch_shapes=(
            [pltpu.VMEM(shape, x.dtype)] * 5 + [pltpu.VMEM(gshape, gamma.dtype)] * 2
        ),
        compiler_params=pltpu.CompilerParams(vmem_limit_bytes=64 * 1024 * 1024),
    )(x.reshape(shape), y.reshape(shape), gamma.reshape(gshape), grad_out.reshape(shape))
    return (out.reshape(x.shape), grad_x.reshape(x.shape), grad_y.reshape(x.shape),
            grad_gamma.reshape(d))
```
